```python
import os as _os
_os.environ.setdefault('JAX_PLATFORMS', 'cpu')
import jax
import jax.numpy as jnp

def _softmax(x, axis=-1):
    return jax.nn.softmax(x, axis=axis)

def _gelu(x):
    return jax.nn.gelu(x, approximate=True)

def _silu(x):
    return jax.nn.silu(x)

def _sigmoid(x):
    return jax.nn.sigmoid(x)

def _layernorm(x, axis=-1, eps=1e-05):
    m = jnp.mean(x, axis=axis, keepdims=True)
    v = jnp.var(x, axis=axis, keepdims=True)
    return (x - m) / jnp.sqrt(v + eps)

def _scatter_add(tgt, idx, src, axis=0):
    return tgt.at[idx].add(src)

def _segment_sum(src, seg, n):
    return jax.ops.segment_sum(src, seg, n)

class _Rng:

    def __init__(self, key):
        self._k = key

    def _next(self):
        self._k, sub = jax.random.split(self._k)
        return sub

    def normal(self, shape):
        return jax.random.normal(self._next(), shape, dtype=jnp.bfloat16)

    def randint(self, lo, hi, shape):
        return jax.random.randint(self._next(), shape, lo, hi, dtype=jnp.int32)

    def uniform(self, shape, lo=0.0, hi=1.0):
        return jax.random.uniform(self._next(), shape, jnp.bfloat16, lo, hi)

    def permutation(self, n):
        return jax.random.permutation(self._next(), n)
kernel_name = 'adaLN_cond__sliding_local_dilated__dense_activation_gelu__prompt'

def setup_inputs():
    _rng = _Rng(jax.random.key(int.from_bytes(__import__("os").urandom(4), "little")))
    _w = lambda a: (lambda t: t.astype(jnp.bfloat16) if jnp.issubdtype(t.dtype, jnp.floating) else t)(jnp.asarray(a))

    def _A_setup():
        B, S, D = (1, 2048, 576)
        return {'x': _w((lambda *s: _rng.normal(s) * 0.05)(B, S, D)), 'wqkv': _w((lambda *s: _rng.normal(s) * 0.05)(D, 3 * D)), 'wo': _w((lambda *s: _rng.normal(s) * 0.05)(D, D))}
    _A_in = _A_setup()

    def _B_setup():
        B, S, D, F = (1, 2048, 576, 4608)
        return {'x': _w((lambda *s: _rng.normal(s) * 0.05)(B, S, D)), 'w1': _w((lambda *s: _rng.normal(s) * 0.8)(D, F) * D ** (-0.5)), 'b1': _w((lambda *s: _rng.normal(s) * 0.8)(F) * 0.01), 'w2': _w((lambda *s: _rng.normal(s) * 0.8)(F, D) * F ** (-0.5)), 'b2': _w((lambda *s: _rng.normal(s) * 0.8)(D) * 0.01)}
    _B_in = _B_setup()
    return {'A_x': _A_in['x'], 'A_wqkv': _A_in['wqkv'], 'A_wo': _A_in['wo'], 'B_x': _B_in['x'], 'B_w1': _B_in['w1'], 'B_b1': _B_in['b1'], 'B_w2': _B_in['w2'], 'B_b2': _B_in['b2'], 'c': _w((lambda *s: _rng.normal(s) * 0.05)(1, 576) * 8.0), 'w_mod': _w((lambda *s: _rng.normal(s) * 0.05)(576, 6 * 576) * 576 ** (-0.5) * 8.0)}

def reference(A_x, A_wqkv, A_wo, B_x, B_w1, B_b1, B_w2, B_b2, c, w_mod):

    def _A_ref(x, wqkv, wo):
        B, S, D = x.shape
        H = 32
        Dh = D // H
        W, dil = (8, 2)
        qkv = (lambda x, *d: x.transpose(*d))((x @ wqkv).reshape(B, S, 3, H, Dh), 2, 0, 3, 1, 4)
        q, k, v = (qkv[0], qkv[1], qkv[2])
        scale = Dh ** (-0.5)
        pos = jnp.arange(S)
        off = jnp.arange(W) * dil
        idx = pos[:, None] - off[None, :]
        mask = idx >= 0
        idx_c = jnp.where(mask, idx, 0).reshape(-1)
        kg = k[:, :, idx_c, :].reshape(B, H, S, W, Dh)
        vg = v[:, :, idx_c, :].reshape(B, H, S, W, Dh)
        logits = jnp.einsum('bhsd,bhswd->bhsw', q, kg) * scale
        logits = jnp.where(mask[None, None, :, :], logits, -1000000000.0)
        attn = _softmax(logits, axis=-1)
        o = jnp.einsum('bhsw,bhswd->bhsd', attn, vg)
        return (lambda x, *d: x.transpose(*d))(o, 0, 2, 1, 3).reshape(B, S, D) @ wo

    def _B_ref(x, w1, b1, w2, b2):
        h = jnp.einsum('bsd,df->bsf', x, w1) + b1
        h = _gelu(h)
        return jnp.einsum('bsf,fd->bsd', h, w2) + b2
    x = A_x
    mod = (_silu(c) @ w_mod).reshape(c.shape[0], 6, 1, -1)
    sa, ca, ga, sb, cb, gb = (mod[:, 0].copy(), mod[:, 1].copy(), mod[:, 2].copy(), mod[:, 3].copy(), mod[:, 4].copy(), mod[:, 5].copy())
    h = _layernorm(x, axis=-1) * (1 + ca) + sa
    x = x + ga * _A_ref(h, A_wqkv, A_wo)
    h = _layernorm(x, axis=-1) * (1 + cb) + sb
    x = x + gb * _B_ref(h, B_w1, B_b1, B_w2, B_b2)
    return x
```

```python
from collections import deque

import jax
import jax.numpy as jnp
import numpy as np
from jax import lax
import jax.experimental.pallas as pl
import jax.experimental.pallas.tpu as pltpu

F32, BF16, U32 = jnp.float32, jnp.bfloat16, jnp.uint32

D, S, FF = 576, 2048, 4608
DH, WIN, DIL = 18, 8, 2
EPS = 1e-5
NQ = S // 512
NP = 2 * NQ
NPART = FF // 512
R = 48
OPS = 7168
GELU_IN = float(np.cbrt(0.044715 * np.sqrt(2.0 / np.pi)))
GELU_LIN = float(np.sqrt(2.0 / np.pi) / GELU_IN)
GELU_OUT = float(0.5 / GELU_IN)
SA, CA, GA, SB, CB, GB, B2 = (i * D for i in range(7))

PRE_A = [lambda a: a(0, 0) + a(1, 1), lambda a: a(1, 0) + a(1, 1), lambda a: a(0, 0), lambda a: a(1, 1),
         lambda a: a(0, 0) + a(0, 1), lambda a: a(1, 0) - a(0, 0), lambda a: a(0, 1) - a(1, 1)]
PRE_B = [lambda b: b(0, 0) - b(1, 1), lambda b: b(0, 0), lambda b: b(1, 1) - b(0, 1), lambda b: b(1, 0) - b(0, 0),
         lambda b: b(1, 1), lambda b: b(0, 0) - b(0, 1), lambda b: b(1, 0) - b(1, 1)]
B_USERS = ((0, 1, 3, 5), (2, 5), (3, 6), (0, 2, 4, 6))
POST_STEPS = {1: ((2, 0), (3, 0)), 3: ((0, 0), (2, 1)), 0: ((0, 1), (3, -1)), 4: ((0, 1), (1, 0)),
              2: ((1, -1), (3, -1)), 5: ((3, -1),), 6: ((0, 1),)}
FLIP = (0, 0, 1, 0, 1, 1, 1)
ROW_PRODUCT = (4, 1)

_BASE = dict(lu=0, ld=1, cap=18, ru=1, rd=1, lead=0.0, ew="oPooPo", oq=(3, 2, 1, 0),
             os=((0, 1, 2), (3, 4, 5, 6)), lag=2, ssa=(8, 0), oo=(0, 1, 2, 5, 3, 4, 6), x=(1,) + (0,) * 9)
MID = dict(var=(1, 1, 1) + (0,) * 9, ops=(0, 0, 0, 1, 1, 1, 1, 1, 0, 1, 1, 2),
           cells=(1, 1, 1, 1, 1, 1, 0, 1, 1, 0, 1, 0), turn=(1, 1, 1, 1, 0, 0, 1, 1, 2, 1, 2, 1),
           units=(2,) * 18 + (3,) * 16, wo=(1,) * 5 + (0,) * 13,
           stats=(2, 2, 2, 1, 2, 2, 0, 0, 0, 0, 0, 1), out=(0,) * 7 + (1, 0, 4, 4, 3))
ORDER = {
    "first": dict(_BASE, cap=12, ru=0, u=(15, 6) + (0,) * 8),
    "plain": dict(_BASE, cap=14, ru=0, rd=0, lead=1.0, ew="oPoooP", oq=(0, 1, 2, 3), os=((2, 5, 1, 0), (3, 4, 6)),
                  oo=(6, 5, 0, 1, 3, 2, 4), c=(0, 3, 0, 1, 1, 2, 2, 3, 1, 8)),
    "up": dict(_BASE, ld=0, ssa=(8, 0, 1), oo=(0, 1, 2, 3, 4, 5, 6), c=(0, 1, 2, 2, 1, 2, 3, 2, 2, 6), wr=16),
    "down": dict(_BASE, lu=1, cap=16, ru=2, rd=0, lead=0.5, ew="ooPoPo", lag=4, ssa=(8,),
                 c=(0, 0, 2, 2, 3, 2, 2, 1, 3, 6), wr=2, xd=(1, 2, 3, 2, 4, 3, 3, 3, 2, 4)),
}


def _post(m):
    return [(m[0] + m[3]) + (m[4] + m[6]), m[4] - m[2], m[1] + m[3], (m[1] - m[0]) - (m[2] + m[5])]


def _two_level(pre, get, o):
    flip = FLIP[o] if pre is PRE_B else 0
    v = [[pre[o](lambda a, b: get(2 * a + i, 2 * b + (j ^ flip))) for j in range(2)] for i in range(2)]
    return [pre[k](lambda i, j: v[i][j]) for k in range(7)]


def _strassen_group(product, emit, cost, lean=0):
    m = {}

    def two():
        m[1], m[3] = product(1), product(3)
        emit(2, m[1] + m[3])

    def five():
        p = product(0)
        a, m[1] = (p + m[3]) + product(6), m[1] - p
        m[4] = product(4)
        emit(0, a + m[4])

    def six():
        p = product(2)
        emit(1, m[4] - p)
        m[1] = m[1] - p

    if lean:
        return [(2 * cost, two), (3 * cost, five), (cost, six), (cost, lambda: emit(3, m[1] - product(5)))]

    def first():
        for i in (0, 1, 2, 5):
            m[i] = product(i)
        emit(3, (m[1] - m[0]) - (m[2] + m[5]))

    def fourth():
        m[3] = product(3)
        emit(2, m[1] + m[3])
        m[0] = m[0] + m[3]

    def fifth():
        m[4] = product(4)
        emit(1, m[4] - m[2])
        m[0] = m[0] + m[4]

    return [(4 * cost, first), (cost, fourth), (cost, fifth), (cost, lambda: emit(0, m[0] + product(6)))]


def _scaled_gelu(z):
    return z + z * jnp.tanh(z * (GELU_LIN + z * z))


def _tree_sum(v):
    while len(v) > 1:
        v = [v[i] + v[i + 1] if i + 1 < len(v) else v[i] for i in range(0, len(v), 2)]
    return v[0]


def _bf(x):
    return pltpu.bitcast(x, BF16)


def _halves(u):
    return pltpu.bitcast(u << 16, F32), pltpu.bitcast(u & np.uint32(0xFFFF0000), F32)


def _mm(a, b):
    return jnp.dot(a, b, preferred_element_type=F32)


def _merge(*streams):
    items = [((k + 0.5) / len(s), si, k, t) for si, s in enumerate(streams) for k, t in enumerate(s)]
    items.sort(key=lambda z: z[:3])
    return [z[3] for z in items]


def _pace(timed, lead, *streams):
    ends = np.cumsum([w for w, _ in timed])
    items = [((e - lead * w) / ends[-1], 0, k, t) for k, (e, (w, t)) in enumerate(zip(ends, timed))]
    items += [((k + 0.5) / len(s), 1 + si, k, t) for si, s in enumerate(streams) for k, t in enumerate(s)]
    items.sort(key=lambda z: z[:3])
    return [z[3] for z in items]


def _split(items, weights):
    ends = np.round(np.cumsum(weights) * len(items) / np.sum(weights)).astype(int).tolist()
    return [items[a:b] for a, b in zip([0] + ends, ends)]


def _run(thunks):
    for t in thunks:
        t()


def _start(*copies):
    for c in copies:
        c.start()


def _wait(*copies):
    for c in copies:
        c.wait()


def _direct(*args):
    return args[-1]


class _Ring:
    def __init__(self, ref, cap):
        self.ref, self.cap, self.free, self.where, self.used = ref, cap, deque(), {}, 0

    def put(self, key, v, recent=False):
        if self.free:
            s = self.free.pop() if recent else self.free.popleft()
        else:
            s, self.used = self.used, self.used + 1
            assert self.used <= self.ref.shape[0]
        self.where[key] = s
        self.ref[s] = v

    def get(self, key, last=True):
        s = self.where[key]
        if last:
            self.drop(key)
        return self.ref[s]

    def drop(self, key):
        self.free.append(self.where.pop(key))
        if len(self.free) > self.cap:
            self.free.popleft()

    def via(self, v):
        self.put("via", v)
        return self.get("via")


def _kernel(x_hbm, wqkv_hbm, wo_hbm, w1_hbm, b1_hbm, w2_hbm, b2_hbm, c_hbm, wmod_hbm, out_hbm,
            x_v, wqkv_v, wo_v, w1_v, w2_v, wmod_v, out_v, modc, wt, wq, wo, hs, hs_next, qs, kv, os_,
            x1, xc, row_sum, w1t, w1s, bias_next, acc, hp, ap, bp, bias, gs, slots, last,
            b1_v, b2_v, c_v, b1f, sem_in, sem_out):
    wq_u, wo_u, kv_u, ap_u = (r.bitcast(U32) for r in (wq, wo, kv, ap))
    lane = lax.broadcasted_iota(jnp.int32, (16, 128), 1)
    lane8 = lax.broadcasted_iota(jnp.int32, (8, 128), 1)

    def cp(i, src, dst):
        return pltpu.make_async_copy(src, dst, sem_in.at[i])

    def cp_cols(i, src, dst, lo, hi):
        return cp(i, src.at[:, lo:hi], dst.at[:, lo:hi])

    mod_cols, qkv_cols = (0, 768, 2 * D, 6 * D), (0, 640, 2 * D, 3 * D)
    cp_c, cp_b1, cp_b2, cp_wo = cp(0, c_hbm, c_v), cp(1, b1_hbm, b1_v), cp(2, b2_hbm, b2_v), cp(3, wo_hbm, wo_v)
    cp_mod = [cp_cols(4 + i, wmod_hbm, wmod_v, *mod_cols[i:i + 2]) for i in range(3)]
    cp_qkv = [cp_cols(7 + i, wqkv_hbm, wqkv_v, *qkv_cols[i:i + 2]) for i in range(3)]
    cp_w1 = [cp(10 + NP + t, w1_hbm.at[:, 512 * t:512 * (t + 1)], w1_v.at[t]) for t in range(NPART)]
    cp_w2 = [cp(10 + NP + NPART + i, w2_hbm.at[:, 1536 * i:1536 * (i + 1)], w2_v.at[i]) for i in range(3)]

    def cp_x(p):
        return cp(10 + p, x_hbm.at[:, pl.ds(pl.multiple_of(256 * p, 256), 256)], x_v.at[p])

    def cp_out(i):
        return pltpu.make_async_copy(out_v.at[i], out_hbm.at[:, pl.ds(pl.multiple_of(512 * i, 512), 512)],
                                     sem_out.at[i])

    def cp_last_rows(k):
        rows = pl.ds(pl.multiple_of(4 * R * k, 16), 4 * R)
        return pltpu.make_async_copy(out_v.at[NQ - 1, rows], out_hbm.at[rows, S - 512:S], sem_out.at[NQ - 1 + k])

    def to_column(row):
        return jnp.broadcast_to(row, (128, row.shape[1])).astype(BF16).T.astype(F32)

    def modulation(lo, hi):
        c = c_v[...].astype(F32)
        act = jnp.broadcast_to(c * jax.nn.sigmoid(c), (16, D)).astype(BF16)
        for n in range(lo, hi, 128):
            col = to_column(_mm(act, wmod_v[:, n:n + 128])[0:1])
            for r in range(n, n + 128, 64):
                m = col[r - n:r - n + 64]
                m = 1.0 + m if r // D * D in (CA, CB) else m
                gain = {SB: GELU_IN, CB: GELU_IN, GB: GELU_OUT}.get(r // D * D)
                modc[r:r + 64, :] = gain * m if gain else m

    def down_bias():
        b2 = b2_v[...].astype(F32).reshape(1, D)
        for n in range(0, D, 128):
            w = min(128, D - n)
            modc[B2 + n:B2 + n + w, :] = to_column(b2[:, n:n + w]) * (1.0 / (3 * GELU_OUT))

    def k_tiles(rows):
        a, b, c = rows(384, 448), rows(448, 512), rows(512, 576)
        return [rows(0, 128), rows(128, 256), rows(256, 384),
                jnp.concatenate([a, b], 0), jnp.concatenate([a, c], 0), jnp.concatenate([c, b], 0)]

    def qkv_row(s, hg, dd):
        return 16 * (hg * 27 + (2 * dd + s if s < 2 else 18 + dd))

    def prep_wqkv(s):
        for n in range(qkv_cols[s], qkv_cols[s + 1], 128):
            w = min(128, 3 * D - n)
            for kt, t in enumerate(k_tiles(lambda a, b: wqkv_v[a:b, n:n + w])):
                wt[kt, n // 2:(n + w) // 2, :] = pltpu.bitcast(t.T, U32)
        for hg in range(4):
            for dd in range(DH // 2):
                for kt in range(6):
                    r0 = qkv_row(s, hg, dd)
                    u = wt[kt, pl.ds(s * 288 + hg * 72 + dd, 8, stride=DH // 2), :]
                    if s == 0:
                        wq[kt, r0:r0 + 16, :] = jnp.concatenate(_halves(u), 0).astype(BF16)
                    else:
                        wq_u[kt, r0 // 2:r0 // 2 + 8, :] = u

    def prep_wo(j):
        n = 128 * j
        w = min(128, D - n)
        wt[j, 0:288, 0:w] = pltpu.bitcast(wo_v[:, n:n + w], U32)
        rows = [jnp.concatenate(_halves(wt[j, pl.ds(hg * 72 + dd, 8, stride=DH // 2), 0:w]), 0)
                for hg in range(4) for dd in range(DH // 2)]
        for kt, t in enumerate(k_tiles(lambda a, b: jnp.concatenate(rows[a // 16:b // 16], 0))):
            wo[kt, n:n + w, :] = t.astype(BF16).T

    def store_pair(dst, r, v1, v2):
        r1 = r if r < 512 else r + 512
        r2 = r + 512 if r < 448 else (r + 640 if r < 512 else r + 448)
        dst[r1:r1 + 16, :] = (v1 - v2 if 448 <= r < 512 else v1).astype(BF16)
        dst[r2:r2 + 16, :] = (v2 - v1 if r >= 512 else v2).astype(BF16)

    def pair_matmul(w, src_u):
        full = [w(0), w(1), w(2)]
        shared = _mm(w(5), _bf(src_u[512:576, :]))
        c1 = _mm(jnp.concatenate(full + [w(3)], 1), _bf(src_u[0:256, :]))
        c2 = _mm(jnp.concatenate(full + [w(4)], 1), _bf(src_u[256:512, :]))
        return c1 + shared, c2 + shared

    def over_rows(s):
        return jnp.broadcast_to(jnp.sum(s, axis=0, keepdims=True) * (1.0 / D), (16, 128))

    def centre(st, j, r0, r1, via=_direct):
        m = via(j, st["mean", j])
        d = [x1[j, r:r + 16, :] - m for r in range(r0, r1, 16)]
        xc[j, r0:r1, :] = jnp.concatenate(d, 0)
        s = _tree_sum([v * v for v in d])
        st[j] = via(j, s if r0 == 0 else st[j] + s)
        if r1 == D:
            st[j] = lax.rsqrt(over_rows(st[j]) + EPS)

    def modulated(st, j, r, scale_at, shift_at):
        return (xc[j, r:r + 16, :] * st[j] * modc[scale_at + r:scale_at + r + 16, :]
                + modc[shift_at + r:shift_at + r + 16, :])

    def ln1(pair, dst):
        st = {}

        def widen(r0, via):
            x = x_v[pair, r0:r0 + 96, :].astype(F32)
            for j in range(2):
                x1[j, r0:r0 + 96, :] = x[:, 128 * j:128 * (j + 1)]
                s = _tree_sum([x[r:r + 16, 128 * j:128 * (j + 1)] for r in range(0, 96, 16)])
                s = s if r0 == 0 else st["mean", j] + s
                st["mean", j] = via(j, over_rows(s) if r0 + 96 == D else s)

        def var(r0, via):
            for j in range(2):
                centre(st, j, r0, r0 + 96, via)

        def out(r0, via):
            rs = {j: via(j, st[j]) for j in range(2)}
            for r in range(r0, r0 + 48, 16):
                v = [modulated(rs, j, r, CA, SA) for j in range(2)]
                store_pair(dst, r, *[via(j, v[j]) if r == r0 + 32 else v[j] for j in range(2)])

        return ([lambda via=_direct, r0=r0: widen(r0, via) for r0 in range(0, D, 96)]
                + [lambda via=_direct, r0=r0: var(r0, via) for r0 in range(0, D, 96)],
                [lambda via=_direct, r0=r0: out(r0, via) for r0 in range(0, D, 48)])

    def ln2(quad):
        st = {("mean", n): over_rows(row_sum[n]) for n in range(4)}

        def var(r0, via):
            for n in range(4):
                centre(st, n, r0, r0 + 48, via)

        def operands(u, via):
            h = {(k, n): via(k, n, modulated(st, n, 128 * k + 16 * u if u < 8 else 512 + 16 * k, CB, SB))
                 for k in range(4) for n in range(4)}
            for o in range(7):
                for i, v in enumerate(_two_level(PRE_B, lambda k, n: h[k, n], o)):
                    hp[quad, pl.ds(144 * (7 * o + i) + 16 * u, 16), :] = v.astype(BF16)

        return ([lambda via=_direct, r0=r0: var(r0, via) for r0 in range(0, D, 48)],
                [lambda via=_direct, u=u: operands(u, via) for u in range(9)])

    def qkv(units):
        def one(group):
            res = pair_matmul(lambda kt: _bf(jnp.concatenate(
                [wq_u[kt, pl.ds(qkv_row(*u) // 2, 8), :] for u in group], 0)), hs.bitcast(U32))
            for i, (s, hg, dd) in enumerate(group):
                for j, v in enumerate(res):
                    if s == 0:
                        qs[j, 9 * hg + dd] = v[16 * i:16 * (i + 1)]
                    else:
                        kv[1 + j, s - 1, 9 * hg + dd] = v[16 * i:16 * (i + 1)].astype(BF16)

        return [lambda i=i: one(units[i:i + R // 16]) for i in range(0, len(units), R // 16)]

    def via_v(i):
        def via(j, v):
            for half in range(2):
                kv_u[1 + j, 1, i + half] = pltpu.bitcast(v[8 * half:8 * (half + 1)], U32)
            return pltpu.bitcast(jnp.concatenate([kv_u[1 + j, 1, i + half] for half in range(2)], 0), F32)

        return via

    def via_q(i):
        def via(j, v):
            qs[j, i] = v
            return qs[j, i]

        return via

    def attend(pair, hg):
        st = {}

        def windows(s, dd):
            u = [kv_u[j, s, 9 * hg + dd] for j in range(3)]
            kv_u[0, s, 9 * hg + dd] = u[2]
            return [[_halves(v) for v in [u[j + 1]] + [
                pltpu.roll(jnp.where(lane8 < 128 - DIL * w, u[j + 1], u[j]), DIL * w, 1)
                for w in range(1, WIN)]] for j in range(2)]

        def scores(dd):
            for j, win in enumerate(windows(0, dd)):
                q = qs[j, 9 * hg + dd]
                st[j] = [(q[0:8] * k0 if dd == 0 else st[j][w] + q[0:8] * k0) + q[8:16] * k1
                         for w, (k0, k1) in enumerate(win)]

        def softmax(j):
            z = [v * (DH ** -0.5) for v in st[j]]
            if j == 0:
                pos = lane8 + 256 * pair
                z = [z[0]] + [jnp.where(pos >= DIL * w, z[w], -1e9) for w in range(1, WIN)]
            m = z[0]
            for v in z[1:]:
                m = jnp.maximum(m, v)
            e = [jnp.exp(v - m) for v in z]
            inv = 1.0 / _tree_sum(e)
            st[j] = [v * inv for v in e]

        def values(dd):
            o = []
            for j, win in enumerate(windows(1, dd)):
                a = [st[j][0] * v for v in win[0]]
                for p, vs in zip(st[j][1:], win[1:]):
                    a = [x + p * v for x, v in zip(a, vs)]
                o.append(jnp.concatenate(a, 0))
            store_pair(os_.at[pair], 16 * (9 * hg + dd), *o)

        return ([lambda dd=dd: scores(dd) for dd in range(DH // 2)] + [lambda: (softmax(0), softmax(1))]
                + [lambda dd=dd: values(dd) for dd in range(DH // 2)])

    def project(quad):
        tot = {}

        def one(r0):
            rows = slice(r0, r0 + R)
            for half in range(2):
                pair = 2 * quad + half
                res = pair_matmul(lambda kt: _bf(wo_u[kt, r0 // 2:(r0 + R) // 2, :]), os_.bitcast(U32).at[pair])
                x = x_v[pair, rows, :].astype(F32)
                for j, v in enumerate(res):
                    n = 2 * j + half
                    y = x[:, 128 * j:128 * (j + 1)] + modc[GA + r0:GA + r0 + R, :] * v
                    x1[n, rows, :] = y
                    acc[quad, n, rows, :] = y
                    s = _tree_sum([y[r:r + 16] for r in range(0, R, 16)])
                    tot[n] = s if r0 == 0 else tot[n] + s
                    if r0 + R == D:
                        row_sum[n] = tot[n]

        return [lambda r0=r0: one(r0) for r0 in range(0, D, R)]

    def transpose_w1(part, dst, t):
        cells, shared_ref, bias_ref = dst

        def one(r, k, via):
            cols = slice(128 * r, 128 * (r + 1))
            main = pltpu.bitcast(w1_v[part, 128 * k:128 * (k + 1), cols].T, U32)
            rem = pltpu.bitcast(jnp.concatenate([w1_v[part, 512 + 16 * k:528 + 16 * k, cols]] * 8, 0).T, U32)
            shared = main[0:8]
            for c in range(8):
                rows = slice(8 * c, 8 * (c + 1))
                cells.bitcast(U32)[t, c, 4 * r + k] = jnp.where((lane8 >> 4) == c, rem[rows], main[rows])
                if c > 0:
                    shared = jnp.where((lane8 >> 4) == c, main[rows], shared)
            shared_ref[t, 4 * r + k] = via(_bf(shared).astype(F32))
            if k == 3:
                col = GELU_IN * to_column(b1f[pl.ds(4 * part + r, 1), :])
                bias_ref[t, r] = jnp.concatenate([col[0:112], via(col[112:128])], 0)

        return [lambda via=_direct, r=r, k=k: one(r, k, via) for r in range(4) for k in range(4)]

    def w1_blocks(cells, shared, t, c):
        if c == 8:
            return [shared[t, i] for i in range(16)]
        return [_bf(cells.bitcast(U32)[t, c, i]).astype(F32) - jnp.where((lane >> 4) == c, 0.0, shared[t, i])
                for i in range(16)]

    def w2_blocks(chunk, t, u):
        w = [w2_v[chunk, pl.ds(4 * R * (u // 3) + R * r + 16 * (u % 3), 16), 512 * t:512 * (t + 1)].astype(F32) for r in range(4)]
        return [w[r][:, 128 * k:128 * (k + 1)] for r in range(4) for k in range(4)]

    def weight_operands(dst, t, row, blocks):
        for o in range(7):
            for i, v in enumerate(_two_level(PRE_A, lambda r, k: blocks[4 * r + k], o)):
                dst[t, pl.ds(144 * (7 * o + i) + row, 16), :] = v.astype(BF16)

    def paced_operands(ring, every, dst, t, row, blocks):
        e = []

        def load():
            e.extend(blocks())
            for i in range(0, 16, every):
                ring.put(("w", t, row, i), e[i])

        def store():
            for i in range(0, 16, every):
                e[i] = ring.get(("w", t, row, i))
            weight_operands(dst, t, row, e)

        return [load, store]

    def up(ring, order, h, g, at, tap=_direct):
        unstaged = {}

        def inner(c, o):
            def product(i):
                p = 7 * o + i
                spans = [(0, 64)] if c == 8 else [(0, 8 * c), (64, 72), (8 * c + 8, 64)]
                rhs = jnp.concatenate([h.bitcast(U32)[72 * p + a:72 * p + b, :] for a, b in spans if a < b], 0)
                lhs = jnp.concatenate([ap_u[t, pl.ds(72 * p + 8 * c, 8), :] for t in range(3)], 0)
                m = _mm(_bf(lhs), _bf(rhs))
                if c < 8 and o in ROW_PRODUCT and i in ROW_PRODUCT:
                    r = 2 * ROW_PRODUCT.index(o) + ROW_PRODUCT.index(i)
                    m = m + jnp.concatenate([bias[t, r, 16 * c:16 * (c + 1), :] for t in range(3)], 0)
                return m

            def emit(q, v):
                for t in range(3):
                    if c in order["ssa"]:
                        unstaged[c, o, q, t] = (tap if (q, t) == (3, 0) else _direct)(v[16 * t:16 * (t + 1)])
                    else:
                        ring.put(("u", c, o, q, t), v[16 * t:16 * (t + 1)], recent=t < order["ru"])

            return _strassen_group(product, lambda q, v: emit(q ^ FLIP[o], v), 1, order["lu"])

        def outer(c, t, q):
            res = _post([unstaged[c, o, q, t] if c in order["ssa"] else ring.get(("u", c, o, q, t))
                         for o in range(7)])
            for z in range(4):
                r, n = 2 * (z // 2) + q // 2, 2 * (z % 2) + q % 2
                if c == 8:
                    ring.put(("s", r, n, t), res[z])
                else:
                    ring.put(("g", t, r, n), _scaled_gelu(res[z] + ring.get(("s", r, n, t), last=c == 7)))

        def operands(c, t, some):
            every = [o for part in order["os"] for o in part]
            for o in some:
                for i, v in enumerate(_two_level(PRE_B, lambda r, n: ring.get(("g", t, r, n), last=False), o)):
                    g[at, 7 * o + i, pl.ds(128 * t + 16 * c, 16), :] = v.astype(BF16)
                for q, users in enumerate(B_USERS):
                    if o == max(users, key=every.index):
                        for z in range(4):
                            ring.drop(("g", t, 2 * (q // 2) + z // 2, 2 * (q % 2) + z % 2))

        cells = [8] + list(range(8))
        th, pending = [], []
        for c in cells:
            for t in range(3):
                four = [lambda c=c, t=t, q=q: outer(c, t, q) for q in order["oq"]]
                for kind in order["ew"]:
                    src = four if kind == "o" else pending
                    th.append(src.pop(0) if src else (lambda: None))
                if c != 8:
                    pending = [lambda c=c, t=t, some=some: operands(c, t, some) for some in order["os"]]
        per = len(th) // 9
        th = [lambda: None] * order["lag"] + th + pending
        return [([inner(cells[k], o) for o in order["oo"]] if k < 9 else [],
                 th[per * (k - 1):per * k if k < 9 else None] if k > 0 else []) for k in range(10)]

    def down_group(w, g, at, row, o, emit, lean=0):
        def product(i):
            p = 7 * o + i
            lhs = jnp.concatenate([_bf(w.bitcast(U32)[t, pl.ds(72 * p + row, R // 2), :]) for t in range(3)], 1)
            m = _mm(lhs, _bf(g.bitcast(U32)[at, p]))
            if o in ROW_PRODUCT and i in ROW_PRODUCT:
                m = m + modc[pl.ds(B2 + R * (2 * ROW_PRODUCT.index(o) + ROW_PRODUCT.index(i)) + 8 * row, R), :]
            return m

        return _strassen_group(product, lambda q, v: emit(q ^ FLIP[o], v), 3, lean)

    def finish(quad, row, get, keep, emit):
        def one(q, j):
            res = get(q, j)
            for ro in range(2):
                r0 = R * (2 * ro + q // 2) + 4 * row + j
                gate = modc[pl.ds(GB + r0, 16), :]
                v = [acc[quad, 2 * co + q % 2, pl.ds(r0, 16), :] + gate * res[2 * ro + co] for co in range(2)]
                for co in range(2) if keep else ():
                    acc[quad, 2 * co + q % 2, pl.ds(r0, 16), :] = v[co]
                if emit:
                    out_v[quad, pl.ds(r0, 16), pl.ds(256 * (q % 2), 256)] = jnp.concatenate(v, 1).astype(BF16)

        return [lambda q=q, j=j: one(q, j) for j in range(0, R, 16) for q in range(4)]

    def down(ring, order, quad, w, g, at, emit_out):
        def finish_rows(k):
            return finish(quad, k * R, lambda q, j: _post([ring.get(("d", k, o, q, j)) for o in range(7)]),
                          True, emit_out)

        def group(k, o):
            def emit(q, v):
                for j in range(0, R, 16):
                    ring.put(("d", k, o, q, j), v[j:j + 16], recent=j < 16 * order["rd"])

            earlier = finish_rows(k - 1)[2 * o:2 * o + 2] if k > 0 else []
            return [(0, t) for t in earlier] + down_group(w, g, at, k * R // 2, o, emit, order["ld"])

        return [group(k, o) for k in range(3) for o in range(7)], finish_rows(2)

    def mlp_step(chunk, quad, g, g_in, g_out, kind):
        order = ORDER[kind]
        ring = _Ring(slots, order["cap"])
        w = bp.at[pl.ds(3 * chunk, 6 if kind == "down" else 3)]
        groups, tail = down(ring, order, NQ - 1 if kind == "down" else quad - 1, w, g, g_in, kind == "plain")
        if kind == "up":
            def blocks(t, c):
                rows = slice(16 * c, 16 * (c + 1))
                for r in range(4) if c < 8 else ():
                    bias[t, r, rows, :] = (bias_next if t else bias)[t or 3, r, rows, :]
                return w1_blocks(w1t, w1s, t or 3, c)

            side = [[]] + [[f for t in range(3) for f in paced_operands(
                ring, order["wr"], ap, t, 16 * c, lambda t=t, c=c: blocks(t, c))] for c in [8] + list(range(8))]
        else:
            turn = transpose_w1(jnp.minimum(3 * chunk + (6 if kind == "down" else 3) + quad, NPART - 1),
                                (w1t, w1s, bias if kind == "down" else bias_next), 3 if kind == "down" else quad)
            side = _split([lambda f=f: f(ring.via) for f in turn], order["x"])
        if kind == "down":
            renew = [f for u in range(9) for t in range(3) for f in paced_operands(
                ring, order["wr"], w, 3 + t, 16 * u, lambda t=t, u=u: w2_blocks(chunk + 1, t, u))]
            side = [_merge(a, b) for a, b in zip(side, _split(renew, order["xd"]))]
        for (mm, ew), a, b in zip(up(ring, order, hp.at[quad], g, g_out), _split(groups, order["c"]), side):
            _run(_pace(sum(_merge(mm, a), [(1e-3, lambda: None)]), order["lead"], ew, b))
        _run(tail)

    def prologue():
        _start(cp_mod[0])
        _wait(cp_c, cp_qkv[0], cp_x(0))
        _start(cp_mod[1])
        stats, out = ln1(0, hs)
        prep_wqkv(0)
        _run(stats)
        _wait(cp_mod[0])
        _start(cp_qkv[1])
        modulation(*mod_cols[0:2])
        _wait(cp_mod[1])
        _start(cp_qkv[2])
        modulation(*mod_cols[1:3])
        _run(out)
        q, k, v = [qkv([(s, hg, dd) for hg in range(4) for dd in range(DH // 2)]) for s in range(3)]
        _run(q[:8])
        _wait(cp_qkv[1])
        _start(cp_x(1))
        prep_wqkv(1)
        _run(q[8:] + k[:8])
        _wait(cp_qkv[2], cp_x(1))
        _start(cp_x(2), cp_x(3), cp_b1, cp_b2)
        prep_wqkv(2)
        _run(k[8:])
        for i, (t, side) in enumerate(zip(v, _split(sum(ln1(1, hs_next), []), [1] * len(v)))):
            for f in side:
                f(via_v(3 * i))
            t()
        for i in range(2 * DH):
            kv_u[0, 1, i] = jnp.broadcast_to(kv_u[1, 1, i][:, 0:1], (8, 128))
        _start(cp_wo, *[cp_x(p) for p in range(4, NP)])

    def attention_pair(p, _):
        pl.when(p < NP - 2)(lambda: _wait(cp_x(p + 2)))
        pl.when(p == 0)(lambda: _start(cp_mod[2], cp_w2[0], *cp_w1[:4]))
        pl.when(p == 3)(lambda: _start(*cp_w2[1:], *cp_w1[4:]))
        hs.bitcast(U32)[...] = hs_next.bitcast(U32)[...]
        stats, out = ln1(jnp.minimum(p + 2, NP - 1), hs_next)
        spots = [(i, via_q, i) for i in range(9)] + [(12 + 3 * i, via_v, 3 * i + 1) for i in range(3)]
        side = {(hg, j): (fs, via(9 * hg + i)) for hg, work, share in ((0, stats, "stats"), (3, out, "out"))
                for (j, via, i), fs in zip(spots, _split(work, MID[share]))}
        for hg in range(4):
            a = attend(p, hg)
            m = qkv(sorted([(s, hg, dd) for s in range(3) for dd in range(DH // 2)], key=lambda u: qkv_row(*u)))
            done = 0
            for i, t in enumerate(m):
                top = 3 * i + 2
                upto = max(top // 2 + 1 if top < 18 else top - 7, min(10, round((i + 1) * len(a) / len(m))))
                for j in range(done, upto):
                    a[j]()
                    fs, via = side.get((hg, j), ([], None))
                    for f in fs:
                        f(via)
                t()
                done = upto

    def first_weights():
        def down_weights(ref, idx, units):
            for t, u in units:
                e = w2_blocks(0, t, u)
                ref[idx] = e[0]
                weight_operands(bp, t, 16 * u, [ref[idx]] + e[1:])

        units = _split([(t, u) for u in range(9) for t in range(3)], MID["units"])
        wo_tiles = _split(list(range(5)), MID["wo"])
        for i, n in enumerate(range(2 * D, 6 * D, 128)):
            for j in wo_tiles[i]:
                prep_wo(j)
            down_weights(modc, (pl.ds(n, 16), slice(None)), units[i])
            modulation(n, n + 128)
        down_bias()
        for i, f in enumerate(transpose_w1(0, (w1t, w1s, bias), 0)):
            down_weights(w1s, (0, i), units[18 + i])
            f()

    def project_next(q, _):
        var, operands = ln2(q)
        groups = project(q + 1)
        var = _split(var, MID["var"])
        operands = _split(operands, MID["ops"])
        view = [r.at[pl.ds(q, 2)] for r in (w1t, w1s, bias)]
        turn = _split(transpose_w1(q + 1, view, 1), MID["turn"])
        cells = _split(list(range(9)), MID["cells"])
        for g, t in enumerate(groups):
            def via(k, n, v):
                if k > 0:
                    return v
                x1[n, R * g:R * g + 16, :] = v
                return x1[n, R * g:R * g + 16, :]

            _run(var[g])
            for c in cells[g]:
                weight_operands(ap, q, 16 * c,
                                [via(i % 4, i // 4, v) for i, v in enumerate(w1_blocks(*view[:2], 0, c))])
            for f in operands[g]:
                f(via)
            for f in turn[g]:
                f(lambda v: via(0, 0, v))
            t()

    def first_step():
        def tap(v):
            qs[0, 0] = v
            return qs[0, 0]

        order = ORDER["first"]
        var, operands = ln2(NQ - 1)
        side = ([lambda f=f: f(lambda n, v: v if n else tap(v)) for f in var]
                + [lambda f=f: f(lambda k, n, v: v if k or n else tap(v)) for f in operands])
        for (mm, ew), a in zip(up(_Ring(slots, order["cap"]), order, hp.at[0], gs, 0, tap), _split(side, order["u"])):
            _run(_pace(sum(mm, [(1e-3, lambda: None)]), order["lead"], ew, a))

    def mlp_chunk(chunk, _):
        def plain_step(quad, _):
            mlp_step(chunk, quad, gs.at[pl.ds(quad - 1, 2)], 0, 1, "plain")
            pl.when(chunk == 2)(lambda: _start(cp_out(quad - 1)))

        lax.fori_loop(1, NQ - 1 + chunk // 2, plain_step, None)
        pl.when(chunk < 2)(lambda: mlp_step(chunk, NQ - 1, gs, NQ - 2, NQ - 1, "up"))
        pl.when(chunk != 2)(lambda: mlp_step(chunk, 0, gs, NQ - 1, 0, "down"))

    def last_rows(k, _):
        def keep(o, q, v):
            for z, sign in POST_STEPS[o]:
                last[q, z] = v if sign == 0 else (last[q, z] + v if sign > 0 else last[q, z] - v)

        for o in POST_STEPS:
            _run([t for _, t in down_group(bp.at[NPART - 3:NPART], gs, NQ - 1, pl.multiple_of(k * (R // 2), 8), o,
                                           lambda q, v: keep(o, q, v))])
        _run(finish(NQ - 1, pl.multiple_of(R * k, 16), lambda q, j: [last[q, z, j:j + 16, :] for z in range(4)],
                    False, True))
        _start(cp_last_rows(k))

    def clear(i, _):
        rows = pl.ds(pl.multiple_of(16 * i, 16), 16)
        kv[0, 0, i] = jnp.zeros((16, 128), BF16)
        for ref in (slots.at[i], qs.at[0, i], x1.at[0, rows], xc.at[0, rows], last.at[0, i % 4, 0:16]):
            ref[...] = jnp.zeros((16, 128), F32)

    _start(cp_c, cp_qkv[0], cp_x(0))
    lax.fori_loop(0, 2 * DH, clear, None)
    prologue()
    lax.fori_loop(0, NP - 1, attention_pair, None)
    _wait(cp_wo, cp_mod[2], cp_b1, cp_b2, cp_w2[0], cp_w1[0])
    b1f[...] = b1_v[...].astype(F32)
    first_weights()
    _wait(*cp_w1[1:4])
    _run(_merge(project(0), [t for hg in range(4) for t in attend(NP - 1, hg)]))
    lax.fori_loop(0, NQ - 1, project_next, None)
    first_step()
    _wait(*cp_w2[1:], *cp_w1[4:])
    lax.fori_loop(0, 3, mlp_chunk, None)
    lax.fori_loop(0, 3, last_rows, None)
    _wait(*[cp_out(i) for i in range(NQ - 1)], *[cp_last_rows(k) for k in range(3)])


@jax.jit
def pallas_adaLN_cond__sliding_local_dilated__dense_activation_gelu__prompt_kernel(
    A_x: jax.Array,
    A_wqkv: jax.Array,
    A_wo: jax.Array,
    B_x: jax.Array,
    B_w1: jax.Array,
    B_b1: jax.Array,
    B_w2: jax.Array,
    B_b2: jax.Array,
    c: jax.Array,
    w_mod: jax.Array,
):
    del B_x
    hbm = pl.BlockSpec(memory_space=pltpu.HBM)
    scratch = [
        pltpu.VMEM((NP, D, 256), BF16),
        pltpu.VMEM((D, 3 * D), BF16),
        pltpu.VMEM((D, D), BF16),
        pltpu.VMEM((NPART, D, 512), BF16),
        pltpu.VMEM((3, D, 1536), BF16),
        pltpu.VMEM((D, 6 * D), BF16),
        pltpu.VMEM((NQ, D, 512), BF16),
        pltpu.VMEM((7 * D, 128), F32),
        pltpu.VMEM((6, 3 * D // 2, 128), U32),
        pltpu.VMEM((6, 3 * D, 128), BF16),
        pltpu.VMEM((6, D, 128), BF16),
        pltpu.VMEM((9 * 128, 128), BF16),
        pltpu.VMEM((9 * 128, 128), BF16),
        pltpu.VMEM((2, 2 * DH, 16, 128), F32),
        pltpu.VMEM((3, 2, 2 * DH, 16, 128), BF16),
        pltpu.VMEM((NP, 9 * 128, 128), BF16),
        pltpu.VMEM((4, D, 128), F32),
        pltpu.VMEM((4, D, 128), F32),
        pltpu.VMEM((4, 16, 128), F32),
        pltpu.VMEM((4, 8, 16, 16, 128), BF16),
        pltpu.VMEM((4, 16, 16, 128), F32),
        pltpu.VMEM((4, 4, 128, 128), F32),
        pltpu.VMEM((NQ, 4, D, 128), F32),
        pltpu.VMEM((NQ, OPS, 128), BF16),
        pltpu.VMEM((3, OPS, 128), BF16),
        pltpu.VMEM((NPART, OPS, 128), BF16),
        pltpu.VMEM((4, 4, 128, 128), F32),
        pltpu.VMEM((NQ, 49, 384, 128), BF16),
        pltpu.VMEM((960, 16, 128), F32),
        pltpu.VMEM((4, 4, R, 128), F32),
        pltpu.VMEM((FF // 128, 128), BF16),
        pltpu.VMEM((D,), BF16),
        pltpu.VMEM((1, D), BF16),
        pltpu.VMEM((FF // 128, 128), F32),
        pltpu.SemaphoreType.DMA((13 + NP + NPART,)),
        pltpu.SemaphoreType.DMA((NQ - 1 + 3,)),
    ]
    out_t = pl.pallas_call(
        _kernel,
        out_shape=jax.ShapeDtypeStruct((D, S), A_x.dtype),
        in_specs=[hbm] * 9,
        out_specs=hbm,
        scratch_shapes=scratch,
        compiler_params=pltpu.CompilerParams(vmem_limit_bytes=126 * 2**20),
        name="adaln_block",
    )(A_x.reshape(S, D).T, A_wqkv, A_wo, B_w1, B_b1.reshape(FF // 128, 128), B_w2.T, B_b2, c, w_mod)
    return out_t.T.reshape(1, S, D)
```
